```python
import os as _os
_os.environ.setdefault("JAX_PLATFORMS", "cpu")
import jax
import jax.numpy as jnp

def _softmax(x, axis=-1):
    return jax.nn.softmax(x, axis=axis)
def _gelu(x):
    return jax.nn.gelu(x, approximate=True)
def _silu(x):
    return jax.nn.silu(x)
def _sigmoid(x):
    return jax.nn.sigmoid(x)
def _layernorm(x, axis=-1, eps=1e-5):
    m = jnp.mean(x, axis=axis, keepdims=True)
    v = jnp.var(x, axis=axis, keepdims=True)
    return (x - m) / jnp.sqrt(v + eps)
def _scatter_add(tgt, idx, src, axis=0):
    return tgt.at[idx].add(src)
def _segment_sum(src, seg, n):
    return jax.ops.segment_sum(src, seg, n)
class _Rng:
    def __init__(self, key):
        self._k = key
    def _next(self):
        self._k, sub = jax.random.split(self._k)
        return sub
    def normal(self, shape):
        return jax.random.normal(self._next(), shape, dtype=jnp.bfloat16)
    def randint(self, lo, hi, shape):
        return jax.random.randint(self._next(), shape, lo, hi, dtype=jnp.int32)
    def uniform(self, shape, lo=0.0, hi=1.0):
        return jax.random.uniform(self._next(), shape, jnp.bfloat16, lo, hi)
    def permutation(self, n):
        return jax.random.permutation(self._next(), n)


kernel_name = 'gated_mix__linear_attn_block__glu_gated_swiglu__prompt'

def setup_inputs():
    _rng = _Rng(jax.random.key(int.from_bytes(__import__("os").urandom(4), "little")))
    _w = (lambda a: (lambda t: t.astype(jnp.bfloat16) if jnp.issubdtype(t.dtype, jnp.floating) else t)(jnp.asarray(a)))
    def _A_setup():
        B, S, D = 1, 2048, 1024
        return {
            "x": _w((lambda *s: _rng.normal(s) * 0.05)(B, S, D)),
            "wqkv": _w((lambda *s: _rng.normal(s) * 0.8)(D, 3 * D)),
            "wo": _w((lambda *s: _rng.normal(s) * 0.05)(D, D)),
        }
    _A_in = _A_setup()

    def _B_setup():
        B, S, D, F = 1, 2048, 1024, 3584
        return {
            "x": _w((lambda *s: _rng.normal(s) * 0.05)(B, S, D)),
            "w1": _w((lambda *s: _rng.normal(s) * 1.6)(D, F) * (2.0 / D) ** 0.5),
            "w3": _w((lambda *s: _rng.normal(s) * 1.6)(D, F) * (2.0 / D) ** 0.5),
            "w2": _w((lambda *s: _rng.normal(s) * 1.6)(F, D) * (2.0 / F) ** 0.5),
        }
    _B_in = _B_setup()

    return {
        "A_x": _A_in["x"],
        "A_wqkv": _A_in["wqkv"],
        "A_wo": _A_in["wo"],
        "B_x": _B_in["x"],
        "B_w1": _B_in["w1"],
        "B_w3": _B_in["w3"],
        "B_w2": _B_in["w2"],
        "gate_w": _w((lambda *s: _rng.normal(s) * 0.05)(1024) * 16.0),
    }

def reference(A_x, A_wqkv, A_wo, B_x, B_w1, B_w3, B_w2, gate_w):
    def _A_ref(x, wqkv, wo):
        B, S, D = x.shape
        H = 32; Dh = D // H
        qkv = (lambda x, *d: x.transpose(*d))((x @ wqkv).reshape(B, S, 3, H, Dh), 2, 0, 3, 1, 4)
        q, k, v = qkv[0], qkv[1], qkv[2]
        phi = lambda t: jnp.where(t > 0, t + 1, jnp.exp(t)) + 1e-6
        pq, pk = phi(q), phi(k)
        kv = jnp.einsum("bhsd,bhse->bhde", pk, v)
        z = jnp.einsum("bhsd->bhd", pk)
        num = jnp.einsum("bhqd,bhde->bhqe", pq, kv)
        den = jnp.einsum("bhqd,bhd->bhq", pq, z)[..., None] + 1e-6
        o = num / den
        return (lambda x, *d: x.transpose(*d))(o, 0, 2, 1, 3).reshape(B, S, D) @ wo

    def _B_ref(x, w1, w3, w2):
        gate = jnp.einsum("bsd,df->bsf", x, w1)
        up = jnp.einsum("bsd,df->bsf", x, w3)
        h = _silu(gate) * up
        out = jnp.einsum("bsf,fd->bsd", h, w2)
        return out

    x = A_x
    g = _sigmoid((x * gate_w).sum(-1, keepdims=True))
    a = _A_ref(x, A_wqkv, A_wo)
    b = _B_ref(x, B_w1, B_w3, B_w2)
    return g * a + (1 - g) * b
```

```python
import functools, contextlib
import numpy as np
import jax
import jax.numpy as jnp
from jax import lax
import jax.experimental.pallas as pl
import jax.experimental.pallas.tpu as pltpu

S, D, F, H, DH = 2048, 1024, 3584, 32, 32
f32, bf16 = jnp.float32, jnp.bfloat16
TM = 256
HM = TM // 2
NB = S // TM
KH = D // 2
FH = F // 2
NJF = FH // 128
NJD = KH // 128

O_KV = 0
O_Q = O_KV + 8 * 5 * 4
O_M = O_Q + NJD * 5 * 4
O_1 = O_M + NJD * 7 * 4
O_3 = O_1 + NJF * 5 * 4
O_2 = O_3 + NJF * 5 * 4
O_X = O_2 + NJD * 5 * NJF
N_TILES = O_X + NB * 5 * NJD

def _phi(t):
    return jnp.where(t > 0, t + 1.0, jnp.exp(t)) + 1e-6

def _silu(t):
    h = 0.5 * t
    return h + h * jnp.tanh(h)

def _dot(a, b):
    return jnp.dot(a, b, preferred_element_type=f32)

def _dot_nt(a, b):
    return lax.dot_general(a, b, (((1,), (1,)), ((), ())), preferred_element_type=f32)

def _dot_tn(a, b):
    return lax.dot_general(a, b, (((0,), (0,)), ((), ())), preferred_element_type=f32)

def combine(M):
    M1, M2, M3, M4, M5, M6, M7 = M
    return (M1 + M4 - M5 + M7, M3 + M5, M2 + M4, M1 - M2 + M3 + M6)

def cat(xs, axis):
    return xs[0] if len(xs) == 1 else jnp.concatenate(xs, axis=axis)

def make(RC=16, vmem_mb=126, scopes=False, flags=None, qpos=(6,8,10,12), xprep_alias=True, u32ld=True, f7=True, tn='f32T', div='rcp', kvdelay=4, qj=4, gw1d=True, finalN=128, b1=(1,4), b2=(4,4), b3=6, b5=2, lag=1, kvA1=4, w1A1=0, w3C0=0, lagA=None, align=True, g5=True, q0=6, qpos0=(9,10,11,12), gwman=True, wqe=False):
    NF = 7 if f7 else 5
    O_KV = 0
    O_Q = O_KV + 8 * NF * 4
    O_M = O_Q + NJD * NF * 4
    O_1 = O_M + NJD * 7 * 4
    O_3 = O_1 + NJF * NF * 4
    O_2 = O_3 + NJF * NF * 4
    O_X = O_2 + NJD * NF * NJF
    O_TOK = O_X + NB * NF * NJD
    N_TILES = O_TOK + 1
    def scope(n):
        return jax.named_scope(n) if scopes else contextlib.nullcontext()

    def kernel(x_hbm, wqkv_hbm, wo_hbm, w1_hbm, w3_hbm, w2_hbm, gw_ref, out_hbm,
               x_v, wq_v, wk_v, wv_v, wo_v, w1_v, w3_v, w2_v,
               tile_v, zt_v, hs_v, pqs_v, pq_v, pkt_v, ob, xsem, wsem, osem, zsem, gwv):
        def xcopy(i):
            return pltpu.make_async_copy(x_hbm.at[pl.ds(i * TM, TM), :], x_v.at[pl.ds(i * TM, TM), :], xsem.at[i])
        def kvcopy(c):
            return [pltpu.make_async_copy(wqkv_hbm.at[:, pl.ds(D + c * 256, 256)], wk_v.at[:, pl.ds(c * 256, 256)], wsem.at[2 * c]),
                    pltpu.make_async_copy(wqkv_hbm.at[:, pl.ds(2 * D + c * 256, 256)], wv_v.at[:, pl.ds(c * 256, 256)], wsem.at[2 * c + 1])]
        def rowcopy(src, dst, r0, n, sk):
            return pltpu.make_async_copy(src.at[pl.ds(r0, n), :], dst.at[pl.ds(r0, n), :], wsem.at[sk])
        NC = 4
        cp_w1 = pltpu.make_async_copy(w1_hbm, w1_v, wsem.at[8])
        cp_w3 = pltpu.make_async_copy(w3_hbm, w3_v, wsem.at[9])
        cp_w2 = pltpu.make_async_copy(w2_hbm, w2_v, wsem.at[10])
        cp_kv23 = [pltpu.make_async_copy(wqkv_hbm.at[:, pl.ds(D + 512, 512)], wk_v.at[:, pl.ds(512, 512)], wsem.at[4]),
                   pltpu.make_async_copy(wqkv_hbm.at[:, pl.ds(2 * D + 512, 512)], wv_v.at[:, pl.ds(512, 512)], wsem.at[5])]
        cp_wq = pltpu.make_async_copy(wqkv_hbm.at[:, pl.ds(0, D)], wq_v, wsem.at[11])
        cp_wo = pltpu.make_async_copy(wo_hbm, wo_v, wsem.at[12])
        def ocopy(i):
            r = pl.ds(i * TM, TM) if isinstance(i, int) else pl.ds(pl.multiple_of(i * TM, TM), TM)
            return pltpu.make_async_copy(ob.at[r, :], out_hbm.at[r, :], osem.at[i])
        def ocopy_c(i, c0, n):
            r = pl.ds(i * TM, TM) if isinstance(i, int) else pl.ds(pl.multiple_of(i * TM, TM), TM)
            return pltpu.make_async_copy(ob.at[r, pl.ds(c0, n)], out_hbm.at[r, pl.ds(c0, n)], osem.at[i])

        xcopy(0).start()
        for c in kvcopy(0): c.start()
        xcopy(1).start()
        if gwman:
            cp_gw = pltpu.make_async_copy(gw_ref, gwv, wsem.at[6])
            cp_gw.start()

        def prep_T_piece(z, base, r1, c1, r2, c2, K, r0):
            nt = K // 128
            b11 = r1[pl.ds(r0, RC), pl.ds(c1, 128)].astype(f32)
            b21 = r1[pl.ds(K + r0, RC), pl.ds(c1, 128)].astype(f32)
            b12 = r2[pl.ds(r0, RC), pl.ds(c2, 128)].astype(f32)
            b22 = r2[pl.ds(K + r0, RC), pl.ds(c2, 128)].astype(f32)
            t = z + base + r0 // 128
            rs = pl.ds(r0 % 128, RC)
            tile_v[t + 0 * nt, rs, :] = (b11 + b22).astype(bf16)
            tile_v[t + 1 * nt, rs, :] = (b12 - b22).astype(bf16)
            tile_v[t + 2 * nt, rs, :] = (b21 - b11).astype(bf16)
            tile_v[t + 3 * nt, rs, :] = (b11 + b12).astype(bf16)
            tile_v[t + 4 * nt, rs, :] = (b21 + b22).astype(bf16)
            if f7:
                tile_v[t + 5 * nt, rs, :] = r1[pl.ds(r0, RC), pl.ds(c1, 128)]
                tile_v[t + 6 * nt, rs, :] = r2[pl.ds(K + r0, RC), pl.ds(c2, 128)]
        def tile(t):
            if u32ld:
                return pltpu.bitcast(tile_v.bitcast(jnp.uint32)[t], bf16)
            return tile_v[t]
        def tload(t, nt):
            return cat([tile(t + u) for u in range(nt)], 0)
        def T_of(base, r1, c1, r2, c2, K):
            nt = K // 128
            if f7:
                return [functools.partial(tload, base + f * nt, nt) for f in (0, 5, 1, 2, 6, 3, 4)]
            return [lambda: tload(base, nt), lambda: r1[pl.ds(0, K), pl.ds(c1, 128)], lambda: tload(base + nt, nt), lambda: tload(base + 2 * nt, nt),
                    lambda: r2[pl.ds(K, K), pl.ds(c2, 128)], lambda: tload(base + 3 * nt, nt), lambda: tload(base + 4 * nt, nt)]
        spec = {
            'kv': lambda j: (O_KV + j * NF * 4, wk_v, j * 128, wv_v, j * 128, KH),
            'q': lambda j: (O_Q + j * NF * 4, wq_v, j * 128, wq_v, KH + j * 128, KH),
            'w1': lambda j: (O_1 + j * NF * 4, w1_v, j * 128, w1_v, FH + j * 128, KH),
            'w3': lambda j: (O_3 + j * NF * 4, w3_v, j * 128, w3_v, FH + j * 128, KH),
            'w2': lambda j: (O_2 + j * NF * NJF, w2_v, j * 128, w2_v, KH + j * 128, FH),
        }
        def T_get(name, j): return T_of(*spec[name](j))
        def prep_pieces(z, name, js):
            out = []
            for j in js:
                sp = spec[name](j)
                for r0 in range(0, sp[-1], RC):
                    out.append(functools.partial(prep_T_piece, z, *sp, r0))
            return out
        def xtile(i, k, p): return O_X + (i * NF + k) * NJD + p
        def prep_x_piece(z, i, p, r0):
            r1 = i * TM; r2 = i * TM + HM
            a11 = x_v[pl.ds(r1 + r0, RC), pl.ds(p * 128, 128)].astype(f32)
            a12 = x_v[pl.ds(r1 + r0, RC), pl.ds(KH + p * 128, 128)].astype(f32)
            a21 = x_v[pl.ds(r2 + r0, RC), pl.ds(p * 128, 128)].astype(f32)
            a22 = x_v[pl.ds(r2 + r0, RC), pl.ds(KH + p * 128, 128)].astype(f32)
            rs = pl.ds(r0, RC)
            zz = z if xprep_alias else 0
            tile_v[zz + xtile(i, 0, p), rs, :] = (a11 + a22).astype(bf16)
            tile_v[zz + xtile(i, 1, p), rs, :] = (a21 + a22).astype(bf16)
            tile_v[zz + xtile(i, 2, p), rs, :] = (a11 + a12).astype(bf16)
            tile_v[zz + xtile(i, 3, p), rs, :] = (a21 - a11).astype(bf16)
            tile_v[zz + xtile(i, 4, p), rs, :] = (a12 - a22).astype(bf16)
            if f7:
                tile_v[zz + xtile(i, 5, p), rs, :] = x_v[pl.ds(r1 + r0, RC), pl.ds(p * 128, 128)]
                tile_v[zz + xtile(i, 6, p), rs, :] = x_v[pl.ds(r2 + r0, RC), pl.ds(KH + p * 128, 128)]
        def prep_x_pieces(z, i):
            return [functools.partial(prep_x_piece, z, i, p, r0) for p in range(NJD) for r0 in range(0, HM, RC)]
        def S_x(i, static):
            if static:
                r1 = pl.ds(i * TM, HM); r2 = pl.ds(i * TM + HM, HM)
            else:
                r1 = pl.ds(pl.multiple_of(i * TM, TM), HM); r2 = pl.ds(pl.multiple_of(i * TM + HM, HM), HM)
            def xs(k): return cat([tile(xtile(i, k, p)) for p in range(NJD)], 1)
            P = functools.partial
            if f7:
                return [P(xs, k) for k in (0, 1, 5, 6, 2, 3, 4)]
            return [P(xs, 0), P(xs, 1), lambda: x_v[r1, pl.ds(0, KH)], lambda: x_v[r2, pl.ds(KH, KH)], P(xs, 2), P(xs, 3), P(xs, 4)]

        rid = lax.broadcasted_iota(jnp.int32, (128, 128), 0) // DH
        cid = lax.broadcasted_iota(jnp.int32, (128, 128), 1) // DH
        bd = rid == cid

        def spread(items, nslots):
            out = [[] for _ in range(nslots)]
            n = len(items)
            for t, it in enumerate(items):
                out[t * nslots // n].append(it)
            return out
        def run(lst):
            for f in lst: f()
        hist = []
        def paced(m, lst, lag=lag):
            hist.append(m)
            if lst and lag > 0 and len(hist) > lag:
                tile_v[O_TOK, pl.ds(0, 16), :] = hist[-1 - lag][:16, :128].astype(bf16)
            run(lst)

        def phaseC(i, static, slots, qj=qj, qpos=qpos):
            r = pl.ds(i * TM, TM) if static else pl.ds(pl.multiple_of(i * TM, TM), TM)
            gw = gwv[...].astype(f32).reshape(1, D) if gwman else (gw_ref[...].astype(f32).reshape(1, D) if gw1d else gw_ref[...].astype(f32))
            g = jax.nn.sigmoid(jnp.sum(x_v[r, :].astype(f32) * gw, axis=-1, keepdims=True))
            g1 = jnp.broadcast_to(g[:HM], (HM, 128)); g2 = jnp.broadcast_to(g[HM:], (HM, 128))
            ng1 = 1.0 - g1; ng2 = 1.0 - g2
            Sx = S_x(i, static)
            sl = [0]
            def slot(m):
                if slots is not None: paced(m, slots[sl[0]])
                sl[0] += 1
            def q_dots(jp):
                Ta = T_get('q', 2 * jp); Tb = T_get('q', 2 * jp + 1)
                M = []
                for k in range(7):
                    M.append(_dot(Sx[k](), cat([Ta[k](), Tb[k]()], 1))); slot(M[-1])
                q11, q12, q21, q22 = combine(M)
                for t in range(2):
                    j = 2 * jp + t
                    cs = slice(t * 128, (t + 1) * 128)
                    pq_v[j] = _phi(cat([q11[:, cs], q21[:, cs]], 0))
                    pq_v[4 + j] = _phi(cat([q12[:, cs], q22[:, cs]], 0))
            def q_norm(j):
                gg = cat([g1, g2], 0)
                if True:
                    p1 = pq_v[j]; p2 = pq_v[4 + j]
                    d1 = _dot_nt(p1.astype(bf16), zt_v[j]) + 1e-6
                    d2 = _dot_nt(p2.astype(bf16), zt_v[4 + j]) + 1e-6
                    if div == 'div':
                        n1 = p1 / d1 * gg; n2 = p2 / d2 * gg
                    else:
                        def rcp(d):
                            r = pl.reciprocal(d, approx=True)
                            return r * (2.0 - d * r)
                        n1 = p1 * (rcp(d1) * gg); n2 = p2 * (rcp(d2) * gg)
                    a11 = n1[:HM]; a21 = n1[HM:]; a12 = n2[:HM]; a22 = n2[HM:]
                    sf = [a11 + a22, a21 + a22, a11, a22, a11 + a12, a21 - a11, a12 - a22]
                    for k in range(7):
                        pqs_v[k, j] = sf[k].astype(bf16)
            def ffn(j):
                Ta = T_get('w1', j); Tb = T_get('w3', j)
                M = []
                for k in range(7):
                    M.append(_dot(Sx[k](), cat([Ta[k](), Tb[k]()], 1))); slot(M[-1])
                C = combine(M)
                h11, h12, h21, h22 = [_silu(c[:, :128]) * c[:, 128:] * ng for c, ng in zip(C, (ng1, ng1, ng2, ng2))]
                hh = [h11 + h22, h21 + h22, h11, h22, h11 + h12, h21 - h11, h12 - h22]
                for k in range(7):
                    hs_v[k, j] = hh[k].astype(bf16)
            for j in range(NJF):
                if j == qj: q_dots(0); q_dots(1)
                if j in qpos: q_norm(qpos.index(j))
                ffn(j)
            T2 = [T_get('w2', j) for j in range(NJD)]
            r1 = pl.ds(i * TM, HM) if static else pl.ds(pl.multiple_of(i * TM, TM), HM)
            r2 = pl.ds(i * TM + HM, HM) if static else pl.ds(pl.multiple_of(i * TM + HM, HM), HM)
            nt = finalN // 128
            for j0 in range(0, NJD, nt):
                M = []
                for k in range(7):
                    lhs = cat([pqs_v[k, j] for j in range(NJD)] + [hs_v[k, j] for j in range(NJF)], 1)
                    rhs = cat([cat([tload(O_M + (j * 7 + k) * 4, 4), T2[j][k]()], 0) for j in range(j0, j0 + nt)], 1)
                    M.append(_dot(lhs, rhs))
                C11, C12, C21, C22 = combine(M)
                c1 = pl.ds(j0 * 128, finalN); c2 = pl.ds(KH + j0 * 128, finalN)
                ob[r1, c1] = C11.astype(bf16)
                ob[r1, c2] = C12.astype(bf16)
                ob[r2, c1] = C21.astype(bf16)
                ob[r2, c2] = C22.astype(bf16)
                if finalN == 512:
                    ocopy(i).start()
                else:
                    ocopy_c(i, j0 * 128, finalN).start()
                    ocopy_c(i, KH + j0 * 128, finalN).start()

        def first(z):
            with scope('wait0'):
                xcopy(0).wait()
                for c in kvcopy(0): c.wait()
                xcopy(1).wait()
            with scope('prep0'):
                for i in (2, 3, 4): xcopy(i).start()
                run(prep_pieces(z, 'kv', [0, 1]))
                run(prep_x_pieces(z, 0))
            kvb = [None] * 8
            def phaseA_pass(p, pre, slots):
                kv = [jnp.zeros((128, 128), f32), jnp.zeros((128, 128), f32)]
                zs = [jnp.zeros((8, 128), f32), jnp.zeros((8, 128), f32)]
                pend = [None]
                def kv_acc():
                    if pend[0] is not None:
                        pkb, vv = pend[0]
                        for t in range(2):
                            cs = slice(t * 128, (t + 1) * 128)
                            if tn == 'lmr':
                                kv[t] = kv[t] + _dot_tn(pkb[:, cs], vv[:, cs])
                            elif tn == 'xpose':
                                kv[t] = kv[t] + _dot(pkb[:, cs].T, vv[:, cs])
                            else:
                                kv[t] = kv[t] + _dot(pkb[t], vv[:, cs])
                        pend[0] = None
                for i in range(NB):
                    run(pre[i])
                    Sx = S_x(i, True)
                    T0 = T_get('kv', 2 * p); T1 = T_get('kv', 2 * p + 1)
                    M = []
                    for k in range(7):
                        M.append(_dot(Sx[k](), cat([T0[k](), T1[k]()], 1)))
                        paced(M[-1], slots[i * 7 + k], lag if lagA is None else lagA)
                        if k == kvdelay: kv_acc()
                    k1, v1, k2, v2 = combine(M)
                    pk = _phi(cat([k1, k2], 0))
                    vv = cat([v1, v2], 0).astype(bf16)
                    for t in range(2):
                        zs[t] = zs[t] + jnp.sum(pk[:, t * 128:(t + 1) * 128].reshape(TM // 8, 8, 128), axis=0)
                    if tn == 'f32T':
                        pend[0] = ([pk[:, t * 128:(t + 1) * 128].T.astype(bf16) for t in range(2)], vv)
                    elif tn == 'refT':
                        for t in range(2):
                            pkt_v[i % 2, t] = pk[:, t * 128:(t + 1) * 128].astype(bf16).T
                        pend[0] = ([pkt_v[i % 2, t] for t in range(2)], vv)
                    else:
                        pend[0] = (pk.astype(bf16), vv)
                kv_acc()
                for t in range(2):
                    g = 2 * p + t
                    kvb[g] = jnp.where(bd, kv[t], 0.0).astype(bf16)
                    zz = jnp.sum(zs[t], axis=0, keepdims=True)
                    zt_v[g] = jnp.where(bd, jnp.broadcast_to(zz, (128, 128)), 0.0).astype(bf16)
            E = lambda: [[] for _ in range(NB)]
            st = lambda c: (lambda: c.start())
            wt = lambda c: (lambda: c.wait())
            def addsl(sl, a, b, items):
                if not items: return
                ps = spread(items, b - a)
                for t in range(a, b): sl[t] = sl[t] + ps[t - a]
            with scope('A0'):
                sl = [[] for _ in range(NB * 7)]
                addsl(sl, 0, 7, prep_x_pieces(z, 1))
                s1 = b1[0] * 7 + b1[1]
                sl[s1] += [wt(xcopy(i)) for i in (2, 3, 4)] + [st(xcopy(i)) for i in (5, 6, 7)] + [st(c) for c in kvcopy(1)]
                addsl(sl, s1 + 1, 14, prep_x_pieces(z, 2))
                addsl(sl, 14, 21, prep_x_pieces(z, 3))
                addsl(sl, 21, 28, prep_x_pieces(z, 4))
                s2 = b2[0] * 7 + b2[1]
                sl[s2] += ([wt(cp_gw)] if gwman else []) + [wt(xcopy(i)) for i in (5, 6, 7)] + [wt(c) for c in kvcopy(1)] + [st(c) for c in cp_kv23] + [st(cp_w1)]
                addsl(sl, s2 + 1, 35, prep_x_pieces(z, 5))
                addsl(sl, 35, 42, prep_x_pieces(z, 6))
                addsl(sl, 42, 49, prep_x_pieces(z, 7))
                addsl(sl, 42, 56, prep_pieces(z, 'kv', [2, 3]))
                phaseA_pass(0, E(), sl)
            with scope('A1'):
                sl = [[] for _ in range(NB * 7)]
                s3 = b3 * 7
                pre = E()
                if align:
                    s3 = -1
                    pre[0] += [wt(c) for c in cp_kv23] + ([st(cp_wq)] if wqe else [])
                else:
                    sl[s3] += [wt(c) for c in cp_kv23] + [wt(cp_w1), st(cp_w3), st(cp_wq)]
                w1p = prep_pieces(z, 'w1', range(NJF)); w3p = prep_pieces(z, 'w3', range(NJF))
                addsl(sl, s3 + 1, 56, prep_pieces(z, 'kv', range(4, 4 + kvA1)) + w1p[:w1A1])
                phaseA_pass(1, pre, sl)
            with scope('A2'):
                sl = [[] for _ in range(NB * 7)]
                addsl(sl, 0, 56, prep_pieces(z, 'kv', range(4 + kvA1, 8)) + w1p[w1A1:])
                pre = E()
                if align: pre[0] += [wt(cp_w1), st(cp_w3)] + ([] if (g5 or wqe) else [st(cp_wq)])
                phaseA_pass(2, pre, sl)
            with scope('A3'):
                pre = E()
                pre[0] += [wt(cp_w3), st(cp_wq), st(cp_wo), st(cp_w2)] if g5 else [wt(cp_w3), wt(cp_wq), st(cp_wo), st(cp_w2)]
                sl = [[] for _ in range(NB * 7)]
                addsl(sl, 0, 56, w3p[:len(w3p) - w3C0])
                phaseA_pass(3, pre, sl)
            def phaseB_g(g):
                m1 = _dot(kvb[g], wo_v[pl.ds(g * 128, 128), :])
                m2 = _dot(kvb[g + 4], wo_v[pl.ds((g + 4) * 128, 128), :])
                for j in range(NJD):
                    b11 = m1[:, j * 128:(j + 1) * 128]; b12 = m1[:, KH + j * 128:KH + (j + 1) * 128]
                    b21 = m2[:, j * 128:(j + 1) * 128]; b22 = m2[:, KH + j * 128:KH + (j + 1) * 128]
                    tf = [b11 + b22, b11, b12 - b22, b21 - b11, b22, b11 + b12, b21 + b22]
                    for k in range(7):
                        tile_v[z + O_M + (j * 7 + k) * 4 + g] = tf[k].astype(bf16)
            with scope('C0'):
                sl = [[] for _ in range(16 * 7)]
                if g5:
                    sl[b5 * 7 - 1] += [wt(cp_wq)]
                    addsl(sl, b5 * 7 + 1, (b5 + 2) * 7, prep_pieces(z, 'q', range(NJD)))
                else:
                    addsl(sl, 0, b5 * 7, prep_pieces(z, 'q', range(NJD)))
                if w3C0:
                    addsl(sl, b5 * 7 + 1, 6 * 7, w3p[len(w3p) - w3C0:])
                sl[b5 * 7 - (1 if g5 else 0)] += [wt(cp_wo), wt(cp_w2)]
                for g in range(4):
                    sl[b5 * 7 + 2 + 4 * g].append(functools.partial(phaseB_g, g))
                addsl(sl, (b5 + 2) * 7, 16 * 7, prep_pieces(z, 'w2', range(NJD)))
                phaseC(0, True, sl, q0, qpos0) if g5 else phaseC(0, True, sl)

        first(pl.semaphore_read(zsem))
        def body(i, c):
            with scope('Ci'):
                phaseC(i, False, None)
            return c
        with scope('loop'):
            lax.fori_loop(1, NB, body, 0)
        with scope('owait'):
            for i in range(NB):
                ocopy(i).wait()

    any_spec = pl.BlockSpec(memory_space=pl.ANY)
    @jax.jit
    def fn(A_x, A_wqkv, A_wo, B_x, B_w1, B_w3, B_w2, gate_w):
        out = pl.pallas_call(
            kernel,
            out_shape=jax.ShapeDtypeStruct((S, D), bf16),
            in_specs=[any_spec] * 6 + [any_spec if gwman else pl.BlockSpec(memory_space=pltpu.VMEM)],
            out_specs=any_spec,
            scratch_shapes=[
                pltpu.VMEM((S, D), bf16),
                pltpu.VMEM((D, D), bf16),
                pltpu.VMEM((D, D), bf16),
                pltpu.VMEM((D, D), bf16),
                pltpu.VMEM((D, D), bf16),
                pltpu.VMEM((D, F), bf16),
                pltpu.VMEM((D, F), bf16),
                pltpu.VMEM((F, D), bf16),
                pltpu.VMEM((N_TILES, 128, 128), bf16),
                pltpu.VMEM((8, 128, 128), bf16),
                pltpu.VMEM((7, NJF, HM, 128), bf16),
                pltpu.VMEM((7, NJD, HM, 128), bf16),
                pltpu.VMEM((8, TM, 128), f32),
                pltpu.VMEM((2, 2, 128, TM), bf16),
                pltpu.VMEM((S, D), bf16),
                pltpu.SemaphoreType.DMA((NB,)),
                pltpu.SemaphoreType.DMA((13,)),
                pltpu.SemaphoreType.DMA((NB,)),
                pltpu.SemaphoreType.REGULAR,
                pltpu.VMEM((D,), bf16),
            ],
            compiler_params=pltpu.CompilerParams(vmem_limit_bytes=vmem_mb * 1024 * 1024, flags=flags),
            name="gmix",
        )(A_x.reshape(S, D), A_wqkv, A_wo, B_w1, B_w3, B_w2, gate_w if gw1d else gate_w.reshape(1, D))
        return out.reshape(1, S, D)
    return fn


_impl = make(lagA=0, b5=3, g5=False, wqe=True)

@jax.jit
def pallas_gated_mix__linear_attn_block__glu_gated_swiglu__prompt_kernel(A_x, A_wqkv, A_wo, B_x, B_w1, B_w3, B_w2, gate_w):
    return _impl(A_x, A_wqkv, A_wo, B_x, B_w1, B_w3, B_w2, gate_w)
```

```python
import functools, contextlib
import numpy as np
import jax
import jax.numpy as jnp
from jax import lax
import jax.experimental.pallas as pl
import jax.experimental.pallas.tpu as pltpu

S, D, F, H, DH = 2048, 1024, 3584, 32, 32
f32, bf16 = jnp.float32, jnp.bfloat16
TM = 256
HM = TM // 2
NB = S // TM
KH = D // 2
FH = F // 2
NJF = FH // 128
NJD = KH // 128

O_KV = 0
O_Q = O_KV + 8 * 5 * 4
O_M = O_Q + NJD * 5 * 4
O_1 = O_M + NJD * 7 * 4
O_3 = O_1 + NJF * 5 * 4
O_2 = O_3 + NJF * 5 * 4
O_X = O_2 + NJD * 5 * NJF
N_TILES = O_X + NB * 5 * NJD

def _phi(t):
    return jnp.where(t > 0, t + 1.0, jnp.exp(t)) + 1e-6

def _silu(t):
    h = 0.5 * t
    return h + h * jnp.tanh(h)

def _dot(a, b):
    return jnp.dot(a, b, preferred_element_type=f32)

def _dot_nt(a, b):
    return lax.dot_general(a, b, (((1,), (1,)), ((), ())), preferred_element_type=f32)

def _dot_tn(a, b):
    return lax.dot_general(a, b, (((0,), (0,)), ((), ())), preferred_element_type=f32)

def combine(M):
    M1, M2, M3, M4, M5, M6, M7 = M
    return (M1 + M4 - M5 + M7, M3 + M5, M2 + M4, M1 - M2 + M3 + M6)

def cat(xs, axis):
    return xs[0] if len(xs) == 1 else jnp.concatenate(xs, axis=axis)

def make(RC=16, vmem_mb=126, scopes=False, flags=None, qpos=(6,8,10,12), xprep_alias=True, u32ld=True, f7=True, tn='f32T', div='rcp', kvdelay=4, qj=4, gw1d=True, finalN=128, b1=(1,4), b2=(4,4), b3=6, b5=3, lag=1, kvA1=4, w1A1=0, w3C0=0, lagA=0, align=True, g5=False, q0=6, qpos0=(9,10,11,12), gwman=True, wqe=True, den='mxu', x1late=False):
    NF = 7 if f7 else 5
    O_KV = 0
    O_Q = O_KV + 8 * NF * 4
    O_M = O_Q + NJD * NF * 4
    O_1 = O_M + NJD * 7 * 4
    O_3 = O_1 + NJF * NF * 4
    O_2 = O_3 + NJF * NF * 4
    O_X = O_2 + NJD * NF * NJF
    O_TOK = O_X + NB * NF * NJD
    N_TILES = O_TOK + 1
    def scope(n):
        return jax.named_scope(n) if scopes else contextlib.nullcontext()

    def kernel(x_hbm, wqkv_hbm, wo_hbm, w1_hbm, w3_hbm, w2_hbm, gw_ref, out_hbm,
               x_v, wq_v, wk_v, wv_v, wo_v, w1_v, w3_v, w2_v,
               tile_v, zt_v, hs_v, pqs_v, pq_v, pkt_v, ob, xsem, wsem, osem, zsem, gwv, zr_v):
        def xcopy(i):
            return pltpu.make_async_copy(x_hbm.at[pl.ds(i * TM, TM), :], x_v.at[pl.ds(i * TM, TM), :], xsem.at[i])
        def kvcopy(c):
            return [pltpu.make_async_copy(wqkv_hbm.at[:, pl.ds(D + c * 256, 256)], wk_v.at[:, pl.ds(c * 256, 256)], wsem.at[2 * c]),
                    pltpu.make_async_copy(wqkv_hbm.at[:, pl.ds(2 * D + c * 256, 256)], wv_v.at[:, pl.ds(c * 256, 256)], wsem.at[2 * c + 1])]
        def rowcopy(src, dst, r0, n, sk):
            return pltpu.make_async_copy(src.at[pl.ds(r0, n), :], dst.at[pl.ds(r0, n), :], wsem.at[sk])
        NC = 4
        cp_w1 = pltpu.make_async_copy(w1_hbm, w1_v, wsem.at[8])
        cp_w3 = pltpu.make_async_copy(w3_hbm, w3_v, wsem.at[9])
        cp_w2 = pltpu.make_async_copy(w2_hbm, w2_v, wsem.at[10])
        cp_kv23 = [pltpu.make_async_copy(wqkv_hbm.at[:, pl.ds(D + 512, 512)], wk_v.at[:, pl.ds(512, 512)], wsem.at[4]),
                   pltpu.make_async_copy(wqkv_hbm.at[:, pl.ds(2 * D + 512, 512)], wv_v.at[:, pl.ds(512, 512)], wsem.at[5])]
        cp_wq = pltpu.make_async_copy(wqkv_hbm.at[:, pl.ds(0, D)], wq_v, wsem.at[11])
        cp_wo = pltpu.make_async_copy(wo_hbm, wo_v, wsem.at[12])
        def ocopy(i):
            r = pl.ds(i * TM, TM) if isinstance(i, int) else pl.ds(pl.multiple_of(i * TM, TM), TM)
            return pltpu.make_async_copy(ob.at[r, :], out_hbm.at[r, :], osem.at[i])
        def ocopy_c(i, c0, n):
            r = pl.ds(i * TM, TM) if isinstance(i, int) else pl.ds(pl.multiple_of(i * TM, TM), TM)
            return pltpu.make_async_copy(ob.at[r, pl.ds(c0, n)], out_hbm.at[r, pl.ds(c0, n)], osem.at[i])

        xcopy(0).start()
        for c in kvcopy(0): c.start()
        xcopy(1).start()
        if gwman:
            cp_gw = pltpu.make_async_copy(gw_ref, gwv, wsem.at[6])
            cp_gw.start()

        def prep_T_piece(z, base, r1, c1, r2, c2, K, r0):
            nt = K // 128
            b11 = r1[pl.ds(r0, RC), pl.ds(c1, 128)].astype(f32)
            b21 = r1[pl.ds(K + r0, RC), pl.ds(c1, 128)].astype(f32)
            b12 = r2[pl.ds(r0, RC), pl.ds(c2, 128)].astype(f32)
            b22 = r2[pl.ds(K + r0, RC), pl.ds(c2, 128)].astype(f32)
            t = z + base + r0 // 128
            rs = pl.ds(r0 % 128, RC)
            tile_v[t + 0 * nt, rs, :] = (b11 + b22).astype(bf16)
            tile_v[t + 1 * nt, rs, :] = (b12 - b22).astype(bf16)
            tile_v[t + 2 * nt, rs, :] = (b21 - b11).astype(bf16)
            tile_v[t + 3 * nt, rs, :] = (b11 + b12).astype(bf16)
            tile_v[t + 4 * nt, rs, :] = (b21 + b22).astype(bf16)
            if f7:
                tile_v[t + 5 * nt, rs, :] = r1[pl.ds(r0, RC), pl.ds(c1, 128)]
                tile_v[t + 6 * nt, rs, :] = r2[pl.ds(K + r0, RC), pl.ds(c2, 128)]
        def tile(t):
            if u32ld:
                return pltpu.bitcast(tile_v.bitcast(jnp.uint32)[t], bf16)
            return tile_v[t]
        def tload(t, nt):
            return cat([tile(t + u) for u in range(nt)], 0)
        def T_of(base, r1, c1, r2, c2, K):
            nt = K // 128
            if f7:
                return [functools.partial(tload, base + f * nt, nt) for f in (0, 5, 1, 2, 6, 3, 4)]
            return [lambda: tload(base, nt), lambda: r1[pl.ds(0, K), pl.ds(c1, 128)], lambda: tload(base + nt, nt), lambda: tload(base + 2 * nt, nt),
                    lambda: r2[pl.ds(K, K), pl.ds(c2, 128)], lambda: tload(base + 3 * nt, nt), lambda: tload(base + 4 * nt, nt)]
        spec = {
            'kv': lambda j: (O_KV + j * NF * 4, wk_v, j * 128, wv_v, j * 128, KH),
            'q': lambda j: (O_Q + j * NF * 4, wq_v, j * 128, wq_v, KH + j * 128, KH),
            'w1': lambda j: (O_1 + j * NF * 4, w1_v, j * 128, w1_v, FH + j * 128, KH),
            'w3': lambda j: (O_3 + j * NF * 4, w3_v, j * 128, w3_v, FH + j * 128, KH),
            'w2': lambda j: (O_2 + j * NF * NJF, w2_v, j * 128, w2_v, KH + j * 128, FH),
        }
        def T_get(name, j): return T_of(*spec[name](j))
        def prep_pieces(z, name, js):
            out = []
            for j in js:
                sp = spec[name](j)
                for r0 in range(0, sp[-1], RC):
                    out.append(functools.partial(prep_T_piece, z, *sp, r0))
            return out
        def xtile(i, k, p): return O_X + (i * NF + k) * NJD + p
        def prep_x_piece(z, i, p, r0):
            r1 = i * TM; r2 = i * TM + HM
            a11 = x_v[pl.ds(r1 + r0, RC), pl.ds(p * 128, 128)].astype(f32)
            a12 = x_v[pl.ds(r1 + r0, RC), pl.ds(KH + p * 128, 128)].astype(f32)
            a21 = x_v[pl.ds(r2 + r0, RC), pl.ds(p * 128, 128)].astype(f32)
            a22 = x_v[pl.ds(r2 + r0, RC), pl.ds(KH + p * 128, 128)].astype(f32)
            rs = pl.ds(r0, RC)
            zz = z if xprep_alias else 0
            tile_v[zz + xtile(i, 0, p), rs, :] = (a11 + a22).astype(bf16)
            tile_v[zz + xtile(i, 1, p), rs, :] = (a21 + a22).astype(bf16)
            tile_v[zz + xtile(i, 2, p), rs, :] = (a11 + a12).astype(bf16)
            tile_v[zz + xtile(i, 3, p), rs, :] = (a21 - a11).astype(bf16)
            tile_v[zz + xtile(i, 4, p), rs, :] = (a12 - a22).astype(bf16)
            if f7:
                tile_v[zz + xtile(i, 5, p), rs, :] = x_v[pl.ds(r1 + r0, RC), pl.ds(p * 128, 128)]
                tile_v[zz + xtile(i, 6, p), rs, :] = x_v[pl.ds(r2 + r0, RC), pl.ds(KH + p * 128, 128)]
        def prep_x_pieces(z, i):
            return [functools.partial(prep_x_piece, z, i, p, r0) for p in range(NJD) for r0 in range(0, HM, RC)]
        def S_x(i, static):
            if static:
                r1 = pl.ds(i * TM, HM); r2 = pl.ds(i * TM + HM, HM)
            else:
                r1 = pl.ds(pl.multiple_of(i * TM, TM), HM); r2 = pl.ds(pl.multiple_of(i * TM + HM, HM), HM)
            def xs(k): return cat([tile(xtile(i, k, p)) for p in range(NJD)], 1)
            P = functools.partial
            if f7:
                return [P(xs, k) for k in (0, 1, 5, 6, 2, 3, 4)]
            return [P(xs, 0), P(xs, 1), lambda: x_v[r1, pl.ds(0, KH)], lambda: x_v[r2, pl.ds(KH, KH)], P(xs, 2), P(xs, 3), P(xs, 4)]

        rid = lax.broadcasted_iota(jnp.int32, (128, 128), 0) // DH
        cid = lax.broadcasted_iota(jnp.int32, (128, 128), 1) // DH
        bd = rid == cid

        def spread(items, nslots):
            out = [[] for _ in range(nslots)]
            n = len(items)
            for t, it in enumerate(items):
                out[t * nslots // n].append(it)
            return out
        def run(lst):
            for f in lst: f()
        hist = []
        def paced(m, lst, lag=lag):
            hist.append(m)
            if lst and lag > 0 and len(hist) > lag:
                tile_v[O_TOK, pl.ds(0, 16), :] = hist[-1 - lag][:16, :128].astype(bf16)
            run(lst)

        def phaseC(i, static, slots, qj=qj, qpos=qpos):
            r = pl.ds(i * TM, TM) if static else pl.ds(pl.multiple_of(i * TM, TM), TM)
            gw = gwv[...].astype(f32).reshape(1, D) if gwman else (gw_ref[...].astype(f32).reshape(1, D) if gw1d else gw_ref[...].astype(f32))
            g = jax.nn.sigmoid(jnp.sum(x_v[r, :].astype(f32) * gw, axis=-1, keepdims=True))
            g1 = jnp.broadcast_to(g[:HM], (HM, 128)); g2 = jnp.broadcast_to(g[HM:], (HM, 128))
            ng1 = 1.0 - g1; ng2 = 1.0 - g2
            Sx = S_x(i, static)
            sl = [0]
            def slot(m):
                if slots is not None: paced(m, slots[sl[0]])
                sl[0] += 1
            def q_dots(jp):
                Ta = T_get('q', 2 * jp); Tb = T_get('q', 2 * jp + 1)
                M = []
                for k in range(7):
                    M.append(_dot(Sx[k](), cat([Ta[k](), Tb[k]()], 1))); slot(M[-1])
                q11, q12, q21, q22 = combine(M)
                for t in range(2):
                    j = 2 * jp + t
                    cs = slice(t * 128, (t + 1) * 128)
                    pq_v[j] = _phi(cat([q11[:, cs], q21[:, cs]], 0))
                    pq_v[4 + j] = _phi(cat([q12[:, cs], q22[:, cs]], 0))
            def q_norm_xlu(c):
                RQ = 32
                lane = lax.broadcasted_iota(jnp.int32, (RQ, 128), 1)
                up = lambda v, t: pltpu.roll(v, t, 1)
                dn = lambda v, t: pltpu.roll(v, 128 - t, 1)
                lo = lambda t: (lane & t) == 0
                def half(r0, gcol):
                    p = [pq_v[g, pl.ds(r0, RQ), :] for g in range(8)]
                    v = [p[g] * zr_v[g] for g in range(8)]
                    for t in (16, 8, 4):
                        v = [jnp.where(lo(t), a, up(b, t)) + jnp.where(lo(t), dn(a, t), b) for a, b in zip(v[0::2], v[1::2])]
                    v = v[0]
                    for t in (2, 1):
                        v = v + jnp.where(lo(t), dn(v, t), up(v, t))
                    v = [gcol / (v + 1e-6)]
                    for t in (4, 8, 16):
                        v = [w for u in v for w in (jnp.where(lo(t), u, up(u, t)), jnp.where(lo(t), dn(u, t), u))]
                    return [p[g] * v[g] for g in range(8)]
                n1 = half(c * RQ, g1[c * RQ:(c + 1) * RQ]); n2 = half(HM + c * RQ, g2[c * RQ:(c + 1) * RQ])
                for j in range(NJD):
                    a11, a12, a21, a22 = n1[j], n1[4 + j], n2[j], n2[4 + j]
                    sf = [a11 + a22, a21 + a22, a11, a22, a11 + a12, a21 - a11, a12 - a22]
                    for k in range(7):
                        pqs_v[k, j, pl.ds(c * RQ, RQ), :] = sf[k].astype(bf16)
            def q_norm(j):
                if den == 'xlu': return q_norm_xlu(j)
                gg = cat([g1, g2], 0)
                if True:
                    p1 = pq_v[j]; p2 = pq_v[4 + j]
                    d1 = _dot_nt(p1.astype(bf16), zt_v[j]) + 1e-6
                    d2 = _dot_nt(p2.astype(bf16), zt_v[4 + j]) + 1e-6
                    if div == 'div':
                        n1 = p1 / d1 * gg; n2 = p2 / d2 * gg
                    else:
                        def rcp(d):
                            r = pl.reciprocal(d, approx=True)
                            return r * (2.0 - d * r)
                        n1 = p1 * (rcp(d1) * gg); n2 = p2 * (rcp(d2) * gg)
                    a11 = n1[:HM]; a21 = n1[HM:]; a12 = n2[:HM]; a22 = n2[HM:]
                    sf = [a11 + a22, a21 + a22, a11, a22, a11 + a12, a21 - a11, a12 - a22]
                    for k in range(7):
                        pqs_v[k, j] = sf[k].astype(bf16)
            def ffn(j):
                Ta = T_get('w1', j); Tb = T_get('w3', j)
                M = []
                for k in range(7):
                    M.append(_dot(Sx[k](), cat([Ta[k](), Tb[k]()], 1))); slot(M[-1])
                C = combine(M)
                h11, h12, h21, h22 = [_silu(c[:, :128]) * c[:, 128:] * ng for c, ng in zip(C, (ng1, ng1, ng2, ng2))]
                hh = [h11 + h22, h21 + h22, h11, h22, h11 + h12, h21 - h11, h12 - h22]
                for k in range(7):
                    hs_v[k, j] = hh[k].astype(bf16)
            for j in range(NJF):
                if j == qj: q_dots(0); q_dots(1)
                if j in qpos: q_norm(qpos.index(j))
                ffn(j)
            T2 = [T_get('w2', j) for j in range(NJD)]
            r1 = pl.ds(i * TM, HM) if static else pl.ds(pl.multiple_of(i * TM, TM), HM)
            r2 = pl.ds(i * TM + HM, HM) if static else pl.ds(pl.multiple_of(i * TM + HM, HM), HM)
            nt = finalN // 128
            for j0 in range(0, NJD, nt):
                M = []
                for k in range(7):
                    lhs = cat([pqs_v[k, j] for j in range(NJD)] + [hs_v[k, j] for j in range(NJF)], 1)
                    rhs = cat([cat([tload(O_M + (j * 7 + k) * 4, 4), T2[j][k]()], 0) for j in range(j0, j0 + nt)], 1)
                    M.append(_dot(lhs, rhs))
                C11, C12, C21, C22 = combine(M)
                c1 = pl.ds(j0 * 128, finalN); c2 = pl.ds(KH + j0 * 128, finalN)
                ob[r1, c1] = C11.astype(bf16)
                ob[r1, c2] = C12.astype(bf16)
                ob[r2, c1] = C21.astype(bf16)
                ob[r2, c2] = C22.astype(bf16)
                if finalN == 512:
                    ocopy(i).start()
                else:
                    ocopy_c(i, j0 * 128, finalN).start()
                    ocopy_c(i, KH + j0 * 128, finalN).start()

        def first(z):
            with scope('wait0'):
                xcopy(0).wait()
                for c in kvcopy(0): c.wait()
                xcopy(1).wait()
            with scope('prep0'):
                for i in (2, 3, 4): xcopy(i).start()
                run(prep_pieces(z, 'kv', [0, 1]))
                run(prep_x_pieces(z, 0))
            kvb = [None] * 8
            def phaseA_pass(p, pre, slots):
                kv = [jnp.zeros((128, 128), f32), jnp.zeros((128, 128), f32)]
                zs = [jnp.zeros((8, 128), f32), jnp.zeros((8, 128), f32)]
                pend = [None]
                def kv_acc():
                    if pend[0] is not None:
                        pkb, vv = pend[0]
                        for t in range(2):
                            cs = slice(t * 128, (t + 1) * 128)
                            if tn == 'lmr':
                                kv[t] = kv[t] + _dot_tn(pkb[:, cs], vv[:, cs])
                            elif tn == 'xpose':
                                kv[t] = kv[t] + _dot(pkb[:, cs].T, vv[:, cs])
                            else:
                                kv[t] = kv[t] + _dot(pkb[t], vv[:, cs])
                        pend[0] = None
                for i in range(NB):
                    run(pre[i])
                    Sx = S_x(i, True)
                    T0 = T_get('kv', 2 * p); T1 = T_get('kv', 2 * p + 1)
                    M = []
                    for k in range(7):
                        M.append(_dot(Sx[k](), cat([T0[k](), T1[k]()], 1)))
                        paced(M[-1], slots[i * 7 + k], lag if lagA is None else lagA)
                        if k == kvdelay: kv_acc()
                    k1, v1, k2, v2 = combine(M)
                    pk = _phi(cat([k1, k2], 0))
                    vv = cat([v1, v2], 0).astype(bf16)
                    for t in range(2):
                        zs[t] = zs[t] + jnp.sum(pk[:, t * 128:(t + 1) * 128].reshape(TM // 8, 8, 128), axis=0)
                    if tn == 'f32T':
                        pend[0] = ([pk[:, t * 128:(t + 1) * 128].T.astype(bf16) for t in range(2)], vv)
                    elif tn == 'refT':
                        for t in range(2):
                            pkt_v[i % 2, t] = pk[:, t * 128:(t + 1) * 128].astype(bf16).T
                        pend[0] = ([pkt_v[i % 2, t] for t in range(2)], vv)
                    else:
                        pend[0] = (pk.astype(bf16), vv)
                kv_acc()
                for t in range(2):
                    g = 2 * p + t
                    kvb[g] = jnp.where(bd, kv[t], 0.0).astype(bf16)
                    zz = jnp.sum(zs[t], axis=0, keepdims=True)
                    if den == 'xlu': zr_v[g] = zz
                    else: zt_v[g] = jnp.where(bd, jnp.broadcast_to(zz, (128, 128)), 0.0).astype(bf16)
            E = lambda: [[] for _ in range(NB)]
            st = lambda c: (lambda: c.start())
            wt = lambda c: (lambda: c.wait())
            def addsl(sl, a, b, items):
                if not items: return
                ps = spread(items, b - a)
                for t in range(a, b): sl[t] = sl[t] + ps[t - a]
            with scope('A0'):
                sl = [[] for _ in range(NB * 7)]
                addsl(sl, 0, 7, prep_x_pieces(z, 1))
                s1 = b1[0] * 7 + b1[1]
                sl[s1] += [wt(xcopy(i)) for i in (2, 3, 4)] + [st(xcopy(i)) for i in (5, 6, 7)] + [st(c) for c in kvcopy(1)]
                addsl(sl, s1 + 1, 14, prep_x_pieces(z, 2))
                addsl(sl, 14, 21, prep_x_pieces(z, 3))
                addsl(sl, 21, 28, prep_x_pieces(z, 4))
                s2 = b2[0] * 7 + b2[1]
                sl[s2] += ([wt(cp_gw)] if gwman else []) + [wt(xcopy(i)) for i in (5, 6, 7)] + [wt(c) for c in kvcopy(1)] + [st(c) for c in cp_kv23] + [st(cp_w1)]
                addsl(sl, s2 + 1, 35, prep_x_pieces(z, 5))
                addsl(sl, 35, 42, prep_x_pieces(z, 6))
                addsl(sl, 42, 49, prep_x_pieces(z, 7))
                addsl(sl, 42, 56, prep_pieces(z, 'kv', [2, 3]))
                phaseA_pass(0, E(), sl)
            with scope('A1'):
                sl = [[] for _ in range(NB * 7)]
                s3 = b3 * 7
                pre = E()
                if align:
                    s3 = -1
                    pre[0] += [wt(c) for c in cp_kv23] + ([st(cp_wq)] if wqe else [])
                else:
                    sl[s3] += [wt(c) for c in cp_kv23] + [wt(cp_w1), st(cp_w3), st(cp_wq)]
                w1p = prep_pieces(z, 'w1', range(NJF)); w3p = prep_pieces(z, 'w3', range(NJF))
                addsl(sl, s3 + 1, 56, prep_pieces(z, 'kv', range(4, 4 + kvA1)) + w1p[:w1A1])
                phaseA_pass(1, pre, sl)
            with scope('A2'):
                sl = [[] for _ in range(NB * 7)]
                addsl(sl, 0, 56, prep_pieces(z, 'kv', range(4 + kvA1, 8)) + w1p[w1A1:])
                pre = E()
                if align: pre[0] += [wt(cp_w1), st(cp_w3)] + ([] if (g5 or wqe) else [st(cp_wq)])
                phaseA_pass(2, pre, sl)
            with scope('A3'):
                pre = E()
                pre[0] += [wt(cp_w3), st(cp_wq), st(cp_wo), st(cp_w2)] if g5 else [wt(cp_w3), wt(cp_wq), st(cp_wo), st(cp_w2)]
                sl = [[] for _ in range(NB * 7)]
                addsl(sl, 0, 56, w3p[:len(w3p) - w3C0])
                phaseA_pass(3, pre, sl)
            def phaseB_g(g):
                m1 = _dot(kvb[g], wo_v[pl.ds(g * 128, 128), :])
                m2 = _dot(kvb[g + 4], wo_v[pl.ds((g + 4) * 128, 128), :])
                for j in range(NJD):
                    b11 = m1[:, j * 128:(j + 1) * 128]; b12 = m1[:, KH + j * 128:KH + (j + 1) * 128]
                    b21 = m2[:, j * 128:(j + 1) * 128]; b22 = m2[:, KH + j * 128:KH + (j + 1) * 128]
                    tf = [b11 + b22, b11, b12 - b22, b21 - b11, b22, b11 + b12, b21 + b22]
                    for k in range(7):
                        tile_v[z + O_M + (j * 7 + k) * 4 + g] = tf[k].astype(bf16)
            with scope('C0'):
                sl = [[] for _ in range(16 * 7)]
                if g5:
                    sl[b5 * 7 - 1] += [wt(cp_wq)]
                    addsl(sl, b5 * 7 + 1, (b5 + 2) * 7, prep_pieces(z, 'q', range(NJD)))
                else:
                    addsl(sl, 0, b5 * 7, prep_pieces(z, 'q', range(NJD)))
                if w3C0:
                    addsl(sl, b5 * 7 + 1, 6 * 7, w3p[len(w3p) - w3C0:])
                sl[b5 * 7 - (1 if g5 else 0)] += [wt(cp_wo), wt(cp_w2)]
                for g in range(4):
                    sl[b5 * 7 + 2 + 4 * g].append(functools.partial(phaseB_g, g))
                addsl(sl, (b5 + 2) * 7, 16 * 7, prep_pieces(z, 'w2', range(NJD)))
                phaseC(0, True, sl, q0, qpos0) if g5 else phaseC(0, True, sl)

        first(pl.semaphore_read(zsem))
        def body(i, c):
            with scope('Ci'):
                phaseC(i, False, None)
            return c
        with scope('loop'):
            lax.fori_loop(1, NB, body, 0)
        with scope('owait'):
            for i in range(NB):
                ocopy(i).wait()

    any_spec = pl.BlockSpec(memory_space=pl.ANY)
    @jax.jit
    def fn(A_x, A_wqkv, A_wo, B_x, B_w1, B_w3, B_w2, gate_w):
        out = pl.pallas_call(
            kernel,
            out_shape=jax.ShapeDtypeStruct((S, D), bf16),
            in_specs=[any_spec] * 6 + [any_spec if gwman else pl.BlockSpec(memory_space=pltpu.VMEM)],
            out_specs=any_spec,
            scratch_shapes=[
                pltpu.VMEM((S, D), bf16),
                pltpu.VMEM((D, D), bf16),
                pltpu.VMEM((D, D), bf16),
                pltpu.VMEM((D, D), bf16),
                pltpu.VMEM((D, D), bf16),
                pltpu.VMEM((D, F), bf16),
                pltpu.VMEM((D, F), bf16),
                pltpu.VMEM((F, D), bf16),
                pltpu.VMEM((N_TILES, 128, 128), bf16),
                pltpu.VMEM((8, 128, 128), bf16),
                pltpu.VMEM((7, NJF, HM, 128), bf16),
                pltpu.VMEM((7, NJD, HM, 128), bf16),
                pltpu.VMEM((8, TM, 128), f32),
                pltpu.VMEM((2, 2, 128, TM), bf16),
                pltpu.VMEM((S, D), bf16),
                pltpu.SemaphoreType.DMA((NB,)),
                pltpu.SemaphoreType.DMA((13,)),
                pltpu.SemaphoreType.DMA((NB,)),
                pltpu.SemaphoreType.REGULAR,
                pltpu.VMEM((D,), bf16),
                pltpu.VMEM((8, 1, 128), f32),
            ],
            compiler_params=pltpu.CompilerParams(vmem_limit_bytes=vmem_mb * 1024 * 1024, flags=flags),
            name="gmix",
        )(A_x.reshape(S, D), A_wqkv, A_wo, B_w1, B_w3, B_w2, gate_w if gw1d else gate_w.reshape(1, D))
        return out.reshape(1, S, D)
    return fn


_impl = make(den='xlu', u32ld=False, f7=False, w3C0=64)

@jax.jit
def pallas_gated_mix__linear_attn_block__glu_gated_swiglu__prompt_kernel(A_x, A_wqkv, A_wo, B_x, B_w1, B_w3, B_w2, gate_w):
    return _impl(A_x, A_wqkv, A_wo, B_x, B_w1, B_w3, B_w2, gate_w)
```
